```python
import jax
import jax.numpy as jnp

def _softmax(x, axis=-1):
    return jax.nn.softmax(x, axis=axis)
def _gelu(x):
    return jax.nn.gelu(x, approximate=True)
def _silu(x):
    return jax.nn.silu(x)
def _sigmoid(x):
    return jax.nn.sigmoid(x)
def _layernorm(x, axis=-1, eps=1e-5):
    m = jnp.mean(x, axis=axis, keepdims=True)
    v = jnp.var(x, axis=axis, keepdims=True)
    return (x - m) / jnp.sqrt(v + eps)
def _scatter_add(tgt, idx, src, axis=0):
    return tgt.at[idx].add(src)
def _segment_sum(src, seg, n):
    return jax.ops.segment_sum(src, seg, n)
class _Rng:
    def __init__(self, key):
        self._k = key
    def _next(self):
        self._k, sub = jax.random.split(self._k)
        return sub
    def normal(self, shape):
        return jax.random.normal(self._next(), shape, dtype=jnp.bfloat16)
    def randint(self, lo, hi, shape):
        return jax.random.randint(self._next(), shape, lo, hi, dtype=jnp.int32)
    def uniform(self, shape, lo=0.0, hi=1.0):
        return jax.random.uniform(self._next(), shape, jnp.bfloat16, lo, hi)
    def permutation(self, n):
        return jax.random.permutation(self._next(), n)


kernel_name = 'standalone__depthwise_separable__vision'

def setup_inputs():
    _rng = _Rng(jax.random.key(int.from_bytes(__import__("os").urandom(4), "little")))
    _w = (lambda a: (lambda t: t.astype(jnp.bfloat16) if jnp.issubdtype(t.dtype, jnp.floating) else t)(jnp.asarray(a)))
    H = W = 384
    C = 384
    k = 1
    return {
        "x": _w((lambda *s: _rng.normal(s) * 0.05)(1, H, W, C)),
        "dw": _w((lambda *s: _rng.normal(s) * 0.05)(k, k, C)),
        "pw": _w((lambda *s: _rng.normal(s) * 0.05)(C, C)),
    }

def reference(x, dw, pw):
    B, H, W, C = x.shape
    k = dw.shape[0]
    pad = k // 2
    xp = jnp.pad(x, ((0,0),(pad,pad),(pad,pad),(0,0)))
    out = jnp.zeros_like(x)
    for i in range(k):
        for j in range(k):
            out = out + xp[:, i:i+H, j:j+W, :] * dw[i, j][None, None, None, :]
    return jnp.einsum('bhwc,cd->bhwd', out, pw)
```

```python
import jax
import jax.numpy as jnp
from jax import lax
import jax.experimental.pallas as pl
import jax.experimental.pallas.tpu as pltpu

_STEP = 1152
_PIECE = 64
_STRIDE = 512
_STREAMS = 4
_AHEAD = 2
_BLOCK = _STRIDE * _STREAMS


def _kernel(x_hbm, dw_hbm, pw_hbm, o_hbm, buf, dw_vmem, pw_vmem, rd_sem, wr_sem, w_sem):
    rows = buf.shape[0]
    n_blocks = rows // _BLOCK
    n_steps = rows // _STEP

    def pieces(block):
        for j in range(_STRIDE // _PIECE):
            for p in range(_STREAMS):
                start = block * _BLOCK + (j * _PIECE + p * _STRIDE)
                if not isinstance(start, int):
                    start = pl.multiple_of(start, _PIECE)
                yield start, p % 2

    def read_block(block):
        for start, queue in pieces(block):
            sl = pl.ds(start, _PIECE)
            pltpu.make_async_copy(
                x_hbm.at[sl], buf.at[sl], rd_sem.at[start // _STEP]
            ).start(priority=queue)

    def write_block(block):
        for start, queue in pieces(block):
            sl = pl.ds(start, _PIECE)
            pltpu.make_async_copy(buf.at[sl], o_hbm.at[sl], wr_sem).start(priority=queue)

    read_block(0)
    dw_copy = pltpu.make_async_copy(dw_hbm, dw_vmem, w_sem.at[0])
    pw_copy = pltpu.make_async_copy(pw_hbm, pw_vmem, w_sem.at[1])
    dw_copy.start()
    pw_copy.start(priority=1)
    for block in range(1, _AHEAD):
        read_block(block)
    dw_copy.wait()
    pw_copy.wait()
    scale = dw_vmem[0].astype(jnp.float32)

    def step(issue):
        def body(s, carry):
            sl = pl.ds(pl.multiple_of(s * _STEP, _STEP), _STEP)
            pltpu.make_async_copy(x_hbm.at[sl], buf.at[sl], rd_sem.at[s]).wait()
            issue(s)
            y = (buf[sl, :].astype(jnp.float32) * scale).astype(buf.dtype)
            buf[sl, :] = jnp.dot(
                y, pw_vmem[...], preferred_element_type=jnp.float32
            ).astype(buf.dtype)
            return carry

        return body

    rd_end = n_blocks - _AHEAD
    wr_end = rd_end
    while (
        wr_end < n_steps
        and wr_end - rd_end < n_blocks
        and (wr_end - rd_end + 1) * _BLOCK <= wr_end * _STEP
    ):
        wr_end += 1

    lax.fori_loop(0, rd_end, step(lambda s: read_block(s + _AHEAD)), None)
    lax.fori_loop(rd_end, wr_end, step(lambda s: write_block(s - rd_end)), None)
    if wr_end < n_steps:
        lax.fori_loop(wr_end, n_steps, step(lambda s: None), None)
    if wr_end - rd_end < n_blocks:
        lax.fori_loop(wr_end - rd_end, n_blocks, lambda b, c: write_block(b), None)
    pltpu.make_async_copy(buf, o_hbm, wr_sem).wait()


@jax.jit
def pallas_standalone__depthwise_separable__vision_kernel(
    x: jax.Array,
    dw: jax.Array,
    pw: jax.Array,
):
    B, H, W, C = x.shape
    rows = B * H * W
    assert dw.shape == (1, 1, C) and pw.shape == (C, C)
    assert rows % _BLOCK == 0 and rows % _STEP == 0 and _STEP % _PIECE == 0

    hbm = pl.BlockSpec(memory_space=pl.ANY)
    out = pl.pallas_call(
        _kernel,
        in_specs=[hbm, hbm, hbm],
        out_specs=hbm,
        out_shape=jax.ShapeDtypeStruct((rows, C), x.dtype),
        scratch_shapes=[
            pltpu.VMEM((rows, C), x.dtype),
            pltpu.VMEM(dw.shape, dw.dtype),
            pltpu.VMEM(pw.shape, pw.dtype),
            pltpu.SemaphoreType.DMA((rows // _STEP,)),
            pltpu.SemaphoreType.DMA(()),
            pltpu.SemaphoreType.DMA((2,)),
        ],
        compiler_params=pltpu.CompilerParams(vmem_limit_bytes=124 * 1024 * 1024),
    )(x.reshape(rows, C), dw, pw)
    return out.reshape(B, H, W, C)
```

```python
import jax
import jax.numpy as jnp
from jax import lax
import jax.experimental.pallas as pl
import jax.experimental.pallas.tpu as pltpu

_STEP = 1024
_PIECE = 64
_STRIDE = 512
_STREAMS = 4
_AHEAD = 3
_PAUSE = 12
_BLOCK = _STRIDE * _STREAMS


def _kernel(x_hbm, dw_hbm, pw_hbm, o_hbm, buf, dw_vmem, pw_vmem, rd_sem, wr_sem):
    rows = buf.shape[0]
    n_blocks = rows // _BLOCK
    n_steps = rows // _STEP

    def pieces(block):
        for j in range(_STRIDE // _PIECE):
            for p in range(_STREAMS):
                start = block * _BLOCK + (j * _PIECE + p * _STRIDE)
                yield pl.ds(pl.multiple_of(start, _PIECE), _PIECE), p % 2

    def read_block(block):
        sem = rd_sem.at[lax.rem(block, _AHEAD)]
        for sl, queue in pieces(block):
            pltpu.make_async_copy(x_hbm.at[sl], buf.at[sl], sem).start(priority=queue)

    def write_block(block):
        for sl, queue in pieces(block):
            pltpu.make_async_copy(buf.at[sl], o_hbm.at[sl], wr_sem).start(priority=queue)

    read_block(jnp.int32(0))
    dw_copy = pltpu.make_async_copy(dw_hbm, dw_vmem, wr_sem)
    pw_copy = pltpu.make_async_copy(pw_hbm, pw_vmem, wr_sem)
    dw_copy.start()
    pw_copy.start(priority=1)
    lax.fori_loop(1, _AHEAD, lambda b, c: read_block(b), None)
    dw_copy.wait()
    pw_copy.wait()
    scale = dw_vmem[0].astype(jnp.float32)

    rd_end = n_blocks - _AHEAD

    def body(s, carry):
        @pl.when(s < n_blocks)
        def _():
            sl = pl.ds(pl.multiple_of(s * _BLOCK, _BLOCK), _BLOCK)
            pltpu.make_async_copy(
                x_hbm.at[sl], buf.at[sl], rd_sem.at[lax.rem(s, _AHEAD)]
            ).wait()

        t = s - rd_end

        @pl.when(t < 0)
        def _():
            read_block(s + _AHEAD)

        @pl.when(jnp.logical_and(t >= 0, lax.rem(t, _PAUSE) != _PAUSE - 1))
        def _():
            write_block(t - lax.div(t, _PAUSE))

        sl = pl.ds(pl.multiple_of(s * _STEP, _STEP), _STEP)
        y = (buf[sl, :].astype(jnp.float32) * scale).astype(buf.dtype)
        buf[sl, :] = jnp.dot(
            y, pw_vmem[...], preferred_element_type=jnp.float32
        ).astype(buf.dtype)
        return carry

    sent = 0
    for s in range(rd_end, n_steps):
        if (s - rd_end) % _PAUSE != _PAUSE - 1:
            assert (sent + 1) * _BLOCK <= s * _STEP
            sent += 1

    lax.fori_loop(0, n_steps, body, None)
    lax.fori_loop(sent, n_blocks, lambda b, c: write_block(b), None)
    pltpu.make_async_copy(buf, o_hbm, wr_sem).wait()


@jax.jit
def pallas_standalone__depthwise_separable__vision_kernel(
    x: jax.Array,
    dw: jax.Array,
    pw: jax.Array,
):
    B, H, W, C = x.shape
    rows = B * H * W
    assert dw.shape == (1, 1, C) and pw.shape == (C, C)
    assert rows % _BLOCK == 0 and rows % _STEP == 0 and _STEP <= _BLOCK

    hbm = pl.BlockSpec(memory_space=pl.ANY)
    out = pl.pallas_call(
        _kernel,
        in_specs=[hbm, hbm, hbm],
        out_specs=hbm,
        out_shape=jax.ShapeDtypeStruct((rows, C), x.dtype),
        scratch_shapes=[
            pltpu.VMEM((rows, C), x.dtype),
            pltpu.VMEM(dw.shape, dw.dtype),
            pltpu.VMEM(pw.shape, pw.dtype),
            pltpu.SemaphoreType.DMA((_AHEAD,)),
            pltpu.SemaphoreType.DMA(()),
        ],
        compiler_params=pltpu.CompilerParams(
            vmem_limit_bytes=124 * 1024 * 1024, disable_bounds_checks=True
        ),
    )(x.reshape(rows, C), dw, pw)
    return out.reshape(B, H, W, C)
```

```python
import jax
import jax.numpy as jnp
from jax import lax
import jax.experimental.pallas as pl
import jax.experimental.pallas.tpu as pltpu

_REGIONS = 12
_SLICE = 192
_BLOCK = _REGIONS * _SLICE
_STEP = _BLOCK // 2
_RD_ROWS = 32
_WR_ROWS = 48
_PARTS = 2
_AHEAD = 3
_CATCH_UP = 6
_ALIGN = 16


def _parts_sent(t, div):
    return _PARTS * t - div(t, _CATCH_UP)


def _kernel(x_hbm, dw_hbm, pw_hbm, o_hbm, buf, dw_vmem, pw_vmem, rd_sem, wr_sem):
    rows = buf.shape[0]
    region = rows // _REGIONS
    n_blocks = rows // _BLOCK
    n_steps = rows // _STEP

    def pieces(hbm_base, vmem_base, size, region_step):
        count = 0
        for j in range(0, _SLICE, size):
            for r in range(0, _REGIONS, region_step):
                in_hbm = pl.multiple_of(hbm_base + (r * region + j), _ALIGN)
                in_vmem = pl.multiple_of(vmem_base + (r * _SLICE + j), _ALIGN)
                yield pl.ds(in_hbm, size), pl.ds(in_vmem, size), count % 2
                count += 1

    def read_block(b, carry=None):
        sem = rd_sem.at[lax.rem(b, _AHEAD)]
        for src, dst, queue in pieces(b * _SLICE, b * _BLOCK, _RD_ROWS, 1):
            pltpu.make_async_copy(x_hbm.at[src], buf.at[dst], sem).start(priority=queue)

    def write_part(p, carry=None):
        b, r0 = lax.div(p, _PARTS), lax.rem(p, _PARTS)
        for dst, src, queue in pieces(
            b * _SLICE + r0 * region, b * _BLOCK + r0 * _SLICE, _WR_ROWS, _PARTS
        ):
            pltpu.make_async_copy(buf.at[src], o_hbm.at[dst], wr_sem).start(priority=queue)

    dw_copy = pltpu.make_async_copy(dw_hbm, dw_vmem, wr_sem)
    pw_copy = pltpu.make_async_copy(pw_hbm, pw_vmem, wr_sem)
    pw_copy.start(priority=1)
    dw_copy.start()
    lax.fori_loop(0, _AHEAD, read_block, None)
    dw_copy.wait()
    pw_copy.wait()
    scale = dw_vmem[0].astype(jnp.float32)

    rd_end = n_blocks - _AHEAD

    def step(s, carry):
        @pl.when(s < n_blocks)
        def _():
            blk = pl.ds(pl.multiple_of(s * _BLOCK, _ALIGN), _BLOCK)
            pltpu.make_async_copy(
                x_hbm.at[blk], buf.at[blk], rd_sem.at[lax.rem(s, _AHEAD)]
            ).wait()

        @pl.when(s < rd_end)
        def _():
            read_block(s + _AHEAD)

        @pl.when(s >= rd_end)
        def _():
            t = s - rd_end
            lax.fori_loop(
                _parts_sent(t, lax.div), _parts_sent(t + 1, lax.div), write_part, None
            )

        sl = pl.ds(pl.multiple_of(s * _STEP, _ALIGN), _STEP)
        y = (buf[sl, :].astype(jnp.float32) * scale).astype(buf.dtype)
        buf[sl, :] = jnp.dot(
            y, pw_vmem[...], preferred_element_type=jnp.float32
        ).astype(buf.dtype)
        return carry

    for s in range(rd_end, n_steps):
        sent = _parts_sent(s + 1 - rd_end, lambda a, b: a // b)
        assert pl.cdiv(sent, _PARTS) * _BLOCK <= s * _STEP

    lax.fori_loop(0, n_steps, step, None)
    lax.fori_loop(sent, n_blocks * _PARTS, write_part, None)
    pltpu.make_async_copy(buf, o_hbm, wr_sem).wait()


@jax.jit
def pallas_standalone__depthwise_separable__vision_kernel(
    x: jax.Array,
    dw: jax.Array,
    pw: jax.Array,
):
    B, H, W, C = x.shape
    rows = B * H * W
    assert dw.shape == (1, 1, C) and pw.shape == (C, C)
    assert rows % _BLOCK == 0 and rows // _BLOCK > _AHEAD

    hbm = pl.BlockSpec(memory_space=pl.ANY)
    out = pl.pallas_call(
        _kernel,
        in_specs=[hbm, hbm, hbm],
        out_specs=hbm,
        out_shape=jax.ShapeDtypeStruct((rows, C), x.dtype),
        scratch_shapes=[
            pltpu.VMEM((rows, C), x.dtype),
            pltpu.VMEM(dw.shape, dw.dtype),
            pltpu.VMEM(pw.shape, pw.dtype),
            pltpu.SemaphoreType.DMA((_AHEAD,)),
            pltpu.SemaphoreType.DMA(()),
        ],
        compiler_params=pltpu.CompilerParams(
            vmem_limit_bytes=120 * 1024 * 1024,
            disable_bounds_checks=True,
        ),
    )(x.reshape(rows, C), dw, pw)
    return out.reshape(B, H, W, C)
```
